```python
import jax
import jax.numpy as jnp

def _softmax(x, axis=-1):
    return jax.nn.softmax(x, axis=axis)

def _gelu(x):
    return jax.nn.gelu(x, approximate=True)

def _silu(x):
    return jax.nn.silu(x)

def _sigmoid(x):
    return jax.nn.sigmoid(x)

def _layernorm(x, axis=-1, eps=1e-05):
    m = jnp.mean(x, axis=axis, keepdims=True)
    v = jnp.var(x, axis=axis, keepdims=True)
    return (x - m) / jnp.sqrt(v + eps)

def _scatter_add(tgt, idx, src, axis=0):
    return tgt.at[idx].add(src)

def _segment_sum(src, seg, n):
    return jax.ops.segment_sum(src, seg, n)

class _Rng:

    def __init__(self, key):
        self._k = key

    def _next(self):
        self._k, sub = jax.random.split(self._k)
        return sub

    def normal(self, shape):
        return jax.random.normal(self._next(), shape, dtype=jnp.bfloat16)

    def randint(self, lo, hi, shape):
        return jax.random.randint(self._next(), shape, lo, hi, dtype=jnp.int32)

    def uniform(self, shape, lo=0.0, hi=1.0):
        return jax.random.uniform(self._next(), shape, jnp.bfloat16, lo, hi)

    def permutation(self, n):
        return jax.random.permutation(self._next(), n)
kernel_name = 'adaLN_cond__sliding_block_cached__mixer_token_mlp__decode'

def setup_inputs():
    _rng = _Rng(jax.random.key(int.from_bytes(__import__("os").urandom(4), "little")))
    _w = lambda a: (lambda t: t.astype(jnp.bfloat16) if jnp.issubdtype(t.dtype, jnp.floating) else t)(jnp.asarray(a))

    def _A_setup():
        B, Sq, D = (1, 1, 640)
        Hq, Hkv, Sk, Dh = (32, 32, 32768, 192)
        assert Hq % Hkv == 0, (Hq, Hkv)
        return {'x': _w((lambda *s: _rng.normal(s) * 0.05)(B, Sq, D)), 'k_cache': _w((lambda *s: _rng.normal(s) * 0.05)(B, Hkv, Sk, Dh)), 'v_cache': _w((lambda *s: _rng.normal(s) * 0.05)(B, Hkv, Sk, Dh)), 'wq': _w((lambda *s: _rng.normal(s) * 0.05)(D, Hq * Dh) * D ** (-0.5)), 'wo': _w((lambda *s: _rng.normal(s) * 0.05)(Hq * Dh, D) * (Hq * Dh) ** (-0.5))}
    _A_in = _A_setup()

    def _B_setup():
        B, S, D, F = (1, 1, 640, 1536)
        return {'x': _w((lambda *s: _rng.normal(s) * 0.05)(B, S, D)), 'w1': _w((lambda *s: _rng.normal(s) * 0.05)(S, F) * S ** (-0.5)), 'b1': _w((lambda *s: _rng.normal(s) * 0.05)(F) * 0.02), 'w2': _w((lambda *s: _rng.normal(s) * 0.05)(F, S) * F ** (-0.5)), 'b2': _w((lambda *s: _rng.normal(s) * 0.05)(S) * 0.02)}
    _B_in = _B_setup()
    return {'A_x': _A_in['x'], 'A_k_cache': _A_in['k_cache'], 'A_v_cache': _A_in['v_cache'], 'A_wq': _A_in['wq'], 'A_wo': _A_in['wo'], 'B_x': _B_in['x'], 'B_w1': _B_in['w1'], 'B_b1': _B_in['b1'], 'B_w2': _B_in['w2'], 'B_b2': _B_in['b2'], 'c': _w((lambda *s: _rng.normal(s) * 0.05)(1, 640)), 'w_mod': _w((lambda *s: _rng.normal(s) * 0.05)(640, 6 * 640) * 640 ** (-0.5))}

def reference(A_x, A_k_cache, A_v_cache, A_wq, A_wo, B_x, B_w1, B_b1, B_w2, B_b2, c, w_mod):

    def _A_ref(x, k_cache, v_cache, wq, wo):
        B, Sq, D = x.shape
        Hq, Dh = (32, 192)
        Hkv, Sk = (k_cache.shape[1], k_cache.shape[2])
        W = min(4096, max(256, Sk // 4))
        rep = Hq // Hkv
        q = (lambda x, *d: x.transpose(*d))((x @ wq).reshape(B, Sq, Hq, Dh), 0, 2, 1, 3)
        k = jnp.repeat(k_cache[:, :, Sk - W:, :], rep, axis=1)
        v = jnp.repeat(v_cache[:, :, Sk - W:, :], rep, axis=1)
        scores = jnp.einsum('bhqd,bhkd->bhqk', q, k) * Dh ** (-0.5)
        p = _softmax(scores, axis=-1)
        o = jnp.einsum('bhqk,bhkd->bhqd', p, v)
        return (lambda x, *d: x.transpose(*d))(o, 0, 2, 1, 3).reshape(B, Sq, Hq * Dh) @ wo

    def _B_ref(x, w1, b1, w2, b2):
        B, S, D = x.shape
        h = _layernorm(x, axis=-1)
        u = jnp.einsum('bsd,sf->bdf', h, w1) + b1
        u = _gelu(u)
        y = jnp.einsum('bdf,fs->bds', u, w2) + b2
        return (lambda x, *d: x.transpose(*d))(y, 0, 2, 1)
    x = A_x
    mod = (_silu(c) @ w_mod).reshape(c.shape[0], 6, 1, -1)
    sa, ca, ga, sb, cb, gb = (mod[:, 0].copy(), mod[:, 1].copy(), mod[:, 2].copy(), mod[:, 3].copy(), mod[:, 4].copy(), mod[:, 5].copy())
    h = _layernorm(x, axis=-1) * (1 + ca) + sa
    x = x + ga * _A_ref(h, A_k_cache, A_v_cache, A_wq, A_wo)
    h = _layernorm(x, axis=-1) * (1 + cb) + sb
    x = x + gb * _B_ref(h, B_w1, B_b1, B_w2, B_b2)
    return x
```

```python
import functools
import math

import jax
import jax.numpy as jnp
import jax.experimental.pallas as pl
import jax.experimental.pallas.tpu as pltpu

D = 640
HQ = 32
DH = 192
F = 1536
G = 2
NBUF = 4
EPS = 1e-5


def _layernorm(x):
    m = jnp.mean(x, axis=-1, keepdims=True)
    xc = x - m
    v = jnp.mean(xc * xc, axis=-1, keepdims=True)
    return xc * jax.lax.rsqrt(v + EPS)


def _mm(a, b):
    return jnp.dot(a, b, preferred_element_type=jnp.float32)


def _kernel(x_hbm, kt_hbm, vt_hbm, wq_hbm, wo_hbm, w1_hbm, b1_hbm, w2_hbm, b2_hbm,
            c_hbm, wmod_hbm, o_ref,
            x_v, c_v, w1_v, b1_v, w2_v, b2_v, wmod_v, wq_v, wo_v, k_v, v_v, q_v,
            sem_s, sem_w, sem_k, sem_v, *, sk, w):
    nstep = HQ // G
    gd = G * DH

    small = [
        pltpu.make_async_copy(c_hbm, c_v, sem_s.at[0]),
        pltpu.make_async_copy(x_hbm, x_v, sem_s.at[1]),
        pltpu.make_async_copy(w1_hbm, w1_v, sem_s.at[2]),
        pltpu.make_async_copy(b1_hbm, b1_v, sem_s.at[3]),
        pltpu.make_async_copy(w2_hbm, w2_v, sem_s.at[4]),
        pltpu.make_async_copy(b2_hbm, b2_v, sem_s.at[5]),
    ]
    cp_mod_a = pltpu.make_async_copy(
        wmod_hbm.at[:, pl.ds(0, 2 * D)], wmod_v.at[:, pl.ds(0, 2 * D)], sem_w.at[0])
    cp_mod_b = pltpu.make_async_copy(
        wmod_hbm.at[:, pl.ds(2 * D, 3 * D)], wmod_v.at[:, pl.ds(2 * D, 3 * D)], sem_w.at[1])
    cp_mod_c = pltpu.make_async_copy(
        wmod_hbm.at[:, pl.ds(5 * D, D)], wmod_v.at[:, pl.ds(5 * D, D)], sem_w.at[2])
    cp_wq = pltpu.make_async_copy(wq_hbm, wq_v, sem_w.at[3])
    cp_wo = pltpu.make_async_copy(wo_hbm, wo_v, sem_w.at[4])

    def cp_k(j, slot):
        return pltpu.make_async_copy(
            kt_hbm.at[pl.ds(j * gd, gd), pl.ds(sk - w, w)], k_v.at[slot], sem_k.at[slot])

    def cp_v(j, slot):
        return pltpu.make_async_copy(
            vt_hbm.at[pl.ds(j * gd, gd), pl.ds(sk - w, w)], v_v.at[slot], sem_v.at[slot])

    small[0].start()
    small[1].start()
    cp_mod_a.start()
    cp_wq.start()
    for s in small[2:]:
        s.start()
    for j in range(NBUF):
        cp_k(j, j).start()
        cp_v(j, j).start()

    small[0].wait()
    cf = c_v[...].astype(jnp.float32)
    sc = cf * jax.nn.sigmoid(cf)
    sc8 = jnp.broadcast_to(sc, (8, D)).astype(jnp.bfloat16)
    cp_mod_a.wait()
    mod_a = _mm(sc8, wmod_v[:, 0:2 * D])[0:1]
    sa, ca = mod_a[:, 0:D], mod_a[:, D:2 * D]
    small[1].wait()
    x0 = x_v[...].astype(jnp.float32)
    h = _layernorm(x0) * (1.0 + ca) + sa
    cp_wq.wait()
    h8 = jnp.broadcast_to(h, (8, D)).astype(jnp.bfloat16)
    q = _mm(h8, wq_v[...]) * (DH ** -0.5)
    row = jax.lax.broadcasted_iota(jnp.int32, (8, gd), 0)
    col = jax.lax.broadcasted_iota(jnp.int32, (8, gd), 1)
    diag = (col >= row * DH) & (col < (row + 1) * DH)
    for j in range(nstep):
        q_v[j] = jnp.where(diag, q[:, j * gd:(j + 1) * gd], 0.0)

    def step(j, acc):
        slot = jax.lax.rem(j, NBUF)
        cp_k(j, slot).wait()
        s = _mm(q_v[j].astype(jnp.bfloat16), k_v[slot])
        m = jnp.max(s, axis=-1, keepdims=True)
        p = jnp.exp(s - m)
        l = jnp.sum(p, axis=-1, keepdims=True)
        cp_v(j, slot).wait()
        o = jax.lax.dot_general(p.astype(jnp.bfloat16), v_v[slot],
                                (((1,), (1,)), ((), ())),
                                preferred_element_type=jnp.float32)
        o = jnp.where(diag, o / l, 0.0)

        @pl.when(j + NBUF < nstep)
        def _():
            cp_k(j + NBUF, slot).start()
            cp_v(j + NBUF, slot).start()

        @pl.when(j == nstep - NBUF)
        def _():
            cp_mod_b.start()
            cp_mod_c.start()

        @pl.when(j == 0)
        def _():
            cp_wo.start()
            cp_wo.wait()

        wo_blk = wo_v[pl.ds(pl.multiple_of(j * gd, gd), gd), :]
        return acc + _mm(o.astype(jnp.bfloat16), wo_blk)

    acc = jax.lax.fori_loop(0, nstep, step, jnp.zeros((8, D), jnp.float32))
    attn = jnp.sum(acc, axis=0, keepdims=True)

    cp_mod_b.wait()
    mod_b = _mm(sc8, wmod_v[:, 2 * D:5 * D])[0:1]
    ga, sb, cb = mod_b[:, 0:D], mod_b[:, D:2 * D], mod_b[:, 2 * D:3 * D]
    x1 = x0 + ga * attn
    h2 = _layernorm(x1) * (1.0 + cb) + sb
    h3 = _layernorm(h2)

    for s_ in small[2:]:
        s_.wait()
    hcol = jnp.transpose(jnp.broadcast_to(h3, (128, D)))
    w1 = w1_v[...].astype(jnp.float32)
    b1 = b1_v[...].astype(jnp.float32)
    w2 = w2_v[...].astype(jnp.float32)
    k0 = math.sqrt(2.0 / math.pi)
    yacc = jnp.zeros((D, 128), jnp.float32)
    for f in range(F // 128):
        sl = slice(f * 128, (f + 1) * 128)
        u = hcol * w1[:, sl] + b1[:, sl]
        g = 0.5 * u * (1.0 + jnp.tanh(k0 * (u + 0.044715 * (u * u * u))))
        yacc = yacc + g * w2[:, sl]
    y = jnp.sum(jnp.transpose(yacc), axis=0, keepdims=True) + b2_v[...].astype(jnp.float32)

    cp_mod_c.wait()
    gb = _mm(sc8, wmod_v[:, 5 * D:6 * D])[0:1]
    o_ref[...] = (x1 + gb * y).astype(o_ref.dtype)


@jax.jit
def pallas_adaLN_cond__sliding_block_cached__mixer_token_mlp__decode_kernel(
    A_x, A_k_cache, A_v_cache, A_wq, A_wo, B_x, B_w1, B_b1, B_w2, B_b2, c, w_mod,
):
    del B_x
    sk = A_k_cache.shape[2]
    w = min(4096, max(256, sk // 4))
    kt = jnp.transpose(A_k_cache, (0, 1, 3, 2)).reshape(HQ * DH, sk)
    vt = jnp.transpose(A_v_cache, (0, 1, 3, 2)).reshape(HQ * DH, sk)
    bf = jnp.bfloat16
    any_spec = pl.BlockSpec(memory_space=pl.ANY)
    out = pl.pallas_call(
        functools.partial(_kernel, sk=sk, w=w),
        in_specs=[any_spec] * 11,
        out_specs=pl.BlockSpec(memory_space=pltpu.VMEM),
        out_shape=jax.ShapeDtypeStruct((1, D), A_x.dtype),
        scratch_shapes=[
            pltpu.VMEM((1, D), bf), pltpu.VMEM((1, D), bf),
            pltpu.VMEM((1, F), bf), pltpu.VMEM((1, F), bf), pltpu.VMEM((1, F), bf),
            pltpu.VMEM((1, 1), bf),
            pltpu.VMEM((D, 6 * D), bf), pltpu.VMEM((D, HQ * DH), bf),
            pltpu.VMEM((HQ * DH, D), bf),
            pltpu.VMEM((NBUF, G * DH, w), bf), pltpu.VMEM((NBUF, G * DH, w), bf),
            pltpu.VMEM((HQ // G, 8, G * DH), jnp.float32),
            pltpu.SemaphoreType.DMA((6,)), pltpu.SemaphoreType.DMA((5,)),
            pltpu.SemaphoreType.DMA((NBUF,)), pltpu.SemaphoreType.DMA((NBUF,)),
        ],
        compiler_params=pltpu.CompilerParams(vmem_limit_bytes=100 * 1024 * 1024),
    )(A_x.reshape(1, D), kt, vt, A_wq, A_wo, B_w1, B_b1.reshape(1, F),
      B_w2.reshape(1, F), B_b2.reshape(1, 1), c, w_mod)
    return out.reshape(A_x.shape)
```

```python
import functools
import math

import jax
import jax.numpy as jnp
import jax.experimental.pallas as pl
import jax.experimental.pallas.tpu as pltpu

D = 640
HQ = 32
DH = 192
F = 1536
G = 2
NBUF = 3
EPS = 1e-5
FB = 128
K0 = math.sqrt(2.0 / math.pi)
S3 = (K0 * 0.044715) ** (1.0 / 3.0)


def _layernorm(x):
    m = jnp.mean(x, axis=-1, keepdims=True)
    xc = x - m
    v = jnp.mean(xc * xc, axis=-1, keepdims=True)
    return xc * jax.lax.rsqrt(v + EPS)


def _mm(a, b):
    return jnp.dot(a, b, preferred_element_type=jnp.float32)


def _kernel(x_hbm, kt_hbm, vt_hbm, wq_hbm, wo_hbm, w1_hbm, b1_hbm, w2_hbm, b2_hbm,
            c_hbm, wmod_hbm, o_ref,
            x_v, c_v, w1_v, b1_v, w2_v, b2_v, wmod_v, wq_v, wo_v, k_v, v_v, q_v, w1c_v, b1c_v,
            sem_s, sem_w, sem_k, sem_v, *, sk, w):
    nstep = HQ // G
    gd = G * DH

    small = [
        pltpu.make_async_copy(c_hbm, c_v, sem_s.at[0]),
        pltpu.make_async_copy(x_hbm, x_v, sem_s.at[1]),
        pltpu.make_async_copy(w1_hbm, w1_v, sem_s.at[2]),
        pltpu.make_async_copy(b1_hbm, b1_v, sem_s.at[3]),
        pltpu.make_async_copy(w2_hbm, w2_v, sem_s.at[4]),
        pltpu.make_async_copy(b2_hbm, b2_v, sem_s.at[5]),
    ]
    cp_mod_a = pltpu.make_async_copy(
        wmod_hbm.at[:, pl.ds(0, 2 * D)], wmod_v.at[:, pl.ds(0, 2 * D)], sem_w.at[0])
    cp_mod = [
        pltpu.make_async_copy(wmod_hbm.at[:, pl.ds(i * D, D)], wmod_v.at[:, pl.ds(i * D, D)],
                              sem_w.at[3 + n])
        for n, i in enumerate((2, 4, 5))]
    cp_sb = [
        pltpu.make_async_copy(wmod_hbm.at[:, pl.ds(3 * D + i * 128, 128)],
                              wmod_v.at[:, pl.ds(3 * D + i * 128, 128)], sem_w.at[6 + i])
        for i in range(D // 128)]
    cp_wq = pltpu.make_async_copy(wq_hbm, wq_v, sem_w.at[1])
    cp_wo = pltpu.make_async_copy(wo_hbm, wo_v, sem_w.at[2])

    def cp_k(j, slot):
        return pltpu.make_async_copy(
            kt_hbm.at[pl.ds(j * gd, gd), pl.ds(sk - w, w)], k_v.at[slot], sem_k.at[slot])

    def cp_v(j, slot):
        return pltpu.make_async_copy(
            vt_hbm.at[pl.ds(j * gd, gd), pl.ds(sk - w, w)], v_v.at[slot], sem_v.at[slot])

    small[0].start()
    small[1].start()
    cp_mod_a.start()
    cp_wq.start()
    cp_wo.start()
    for s in small[2:]:
        s.start()
    for j in range(NBUF):
        cp_k(j, j).start()
        cp_v(j, j).start()

    small[0].wait()
    cf = c_v[...].astype(jnp.float32)
    sc = cf * jax.nn.sigmoid(cf)
    sc8 = jnp.broadcast_to(sc, (8, D)).astype(jnp.bfloat16)
    cp_mod_a.wait()
    mod_a = _mm(sc8, wmod_v[:, 0:2 * D])[0:1]
    sa, ca = mod_a[:, 0:D], mod_a[:, D:2 * D]
    small[1].wait()
    x0 = x_v[...].astype(jnp.float32)
    h = _layernorm(x0) * (1.0 + ca) + sa
    cp_wq.wait()
    h8 = jnp.broadcast_to(h, (8, D)).astype(jnp.bfloat16)
    q = _mm(h8, wq_v[...]) * (DH ** -0.5)
    row = jax.lax.broadcasted_iota(jnp.int32, (8, gd), 0)
    col = jax.lax.broadcasted_iota(jnp.int32, (8, gd), 1)
    diag = (col >= row * DH) & (col < (row + 1) * DH)
    for j in range(nstep):
        q_v[j] = jnp.where(diag, q[:, j * gd:(j + 1) * gd], 0.0)

    for s_ in small[2:]:
        s_.wait()
    w1c_v[...] = jnp.transpose(jnp.broadcast_to(w1_v[...].astype(jnp.float32) * S3, (128, F)))
    b1c_v[...] = jnp.transpose(jnp.broadcast_to(
        b1_v[...].astype(jnp.float32).reshape(1, F) * S3, (128, F)))
    w2b = jnp.broadcast_to(w2_v[...].astype(jnp.float32), (8, F))

    def step(j, acc):
        slot = jax.lax.rem(j, NBUF)
        cp_k(j, slot).wait()
        s = _mm(q_v[j].astype(jnp.bfloat16), k_v[slot])
        m = jnp.max(s, axis=-1, keepdims=True)
        p = jnp.exp(s - m)
        l = jnp.sum(p, axis=-1, keepdims=True)
        cp_v(j, slot).wait()
        o = jax.lax.dot_general(p.astype(jnp.bfloat16), v_v[slot],
                                (((1,), (1,)), ((), ())),
                                preferred_element_type=jnp.float32)
        o = jnp.where(diag, o / l, 0.0)

        @pl.when(j + NBUF < nstep)
        def _():
            cp_k(j + NBUF, slot).start()
            cp_v(j + NBUF, slot).start()

        @pl.when(j == nstep - NBUF)
        def _():
            for cp in cp_mod[:2] + cp_sb + cp_mod[2:]:
                cp.start()

        wo_blk = wo_v[pl.ds(pl.multiple_of(j * gd, gd), gd), :]
        return acc + _mm(o.astype(jnp.bfloat16), wo_blk)

    cp_wo.wait()
    acc = jax.lax.fori_loop(0, nstep, step, jnp.zeros((8, D), jnp.float32))
    attn = jnp.sum(acc, axis=0, keepdims=True)

    cp_mod[0].wait()
    ga = _mm(sc8, wmod_v[:, 2 * D:3 * D])[0:1]
    x1 = x0 + ga * attn
    ln1 = _layernorm(x1)
    cp_mod[1].wait()
    cb = _mm(sc8, wmod_v[:, 4 * D:5 * D])[0:1]
    h2 = ln1 * (1.0 + cb)
    sbs = []
    for i in range(D // 128):
        cp_sb[i].wait()
        sbs.append(_mm(sc8, wmod_v[:, 3 * D + i * 128:3 * D + (i + 1) * 128])[0:1])
    h3 = _layernorm(h2 + jnp.concatenate(sbs, axis=-1))

    y = jnp.zeros((8, D), jnp.float32)
    nfb = F // FB
    for f in range(nfb):
        if f == nfb // 2:
            cp_mod[2].wait()
            gb = _mm(sc8, wmod_v[:, 5 * D:6 * D])[0:1]
        w1c = w1c_v[f * FB:(f + 1) * FB, :]
        b1c = b1c_v[f * FB:(f + 1) * FB, :]
        gs = []
        for i in range(D // 128):
            us = w1c * h3[:, i * 128:(i + 1) * 128] + b1c
            t = jnp.tanh(us * (us * us + (K0 / S3)))
            gs.append(us * t + us)
        y = y + _mm(w2b[:, f * FB:(f + 1) * FB], jnp.concatenate(gs, axis=-1))
    y = y[0:1] * (0.5 / S3) + b2_v[...].astype(jnp.float32)
    o_ref[...] = (x1 + gb * y).astype(o_ref.dtype)


@jax.jit
def pallas_adaLN_cond__sliding_block_cached__mixer_token_mlp__decode_kernel(
    A_x, A_k_cache, A_v_cache, A_wq, A_wo, B_x, B_w1, B_b1, B_w2, B_b2, c, w_mod,
):
    del B_x
    sk = A_k_cache.shape[2]
    w = min(4096, max(256, sk // 4))
    kt = jnp.transpose(A_k_cache, (0, 1, 3, 2)).reshape(HQ * DH, sk)
    vt = jnp.transpose(A_v_cache, (0, 1, 3, 2)).reshape(HQ * DH, sk)
    bf = jnp.bfloat16
    any_spec = pl.BlockSpec(memory_space=pl.ANY)
    out = pl.pallas_call(
        functools.partial(_kernel, sk=sk, w=w),
        in_specs=[any_spec] * 11,
        out_specs=pl.BlockSpec(memory_space=pltpu.VMEM),
        out_shape=jax.ShapeDtypeStruct((1, D), A_x.dtype),
        scratch_shapes=[
            pltpu.VMEM((1, D), bf), pltpu.VMEM((1, D), bf),
            pltpu.VMEM((1, F), bf), pltpu.VMEM((F,), bf), pltpu.VMEM((1, F), bf),
            pltpu.VMEM((1, 1), bf),
            pltpu.VMEM((D, 6 * D), bf), pltpu.VMEM((D, HQ * DH), bf),
            pltpu.VMEM((HQ * DH, D), bf),
            pltpu.VMEM((NBUF, G * DH, w), bf), pltpu.VMEM((NBUF, G * DH, w), bf),
            pltpu.VMEM((HQ // G, 8, G * DH), jnp.float32),
            pltpu.VMEM((F, 128), jnp.float32), pltpu.VMEM((F, 128), jnp.float32),
            pltpu.SemaphoreType.DMA((6,)), pltpu.SemaphoreType.DMA((11,)),
            pltpu.SemaphoreType.DMA((NBUF,)), pltpu.SemaphoreType.DMA((NBUF,)),
        ],
        compiler_params=pltpu.CompilerParams(vmem_limit_bytes=100 * 1024 * 1024),
    )(A_x.reshape(1, D), kt, vt, A_wq, A_wo, B_w1, B_b1,
      B_w2.reshape(1, F), B_b2.reshape(1, 1), c, w_mod)
    return out.reshape(A_x.shape)
```
